```python
import os as _os
_os.environ.setdefault("JAX_PLATFORMS", "cpu")
import jax
import jax.numpy as jnp

def _softmax(x, axis=-1):
    return jax.nn.softmax(x, axis=axis)
def _gelu(x):
    return jax.nn.gelu(x, approximate=True)
def _silu(x):
    return jax.nn.silu(x)
def _sigmoid(x):
    return jax.nn.sigmoid(x)
def _layernorm(x, axis=-1, eps=1e-5):
    m = jnp.mean(x, axis=axis, keepdims=True)
    v = jnp.var(x, axis=axis, keepdims=True)
    return (x - m) / jnp.sqrt(v + eps)
def _scatter_add(tgt, idx, src, axis=0):
    return tgt.at[idx].add(src)
def _segment_sum(src, seg, n):
    return jax.ops.segment_sum(src, seg, n)
class _Rng:
    def __init__(self, key):
        self._k = key
    def _next(self):
        self._k, sub = jax.random.split(self._k)
        return sub
    def normal(self, shape):
        return jax.random.normal(self._next(), shape, dtype=jnp.bfloat16)
    def randint(self, lo, hi, shape):
        return jax.random.randint(self._next(), shape, lo, hi, dtype=jnp.int32)
    def uniform(self, shape, lo=0.0, hi=1.0):
        return jax.random.uniform(self._next(), shape, jnp.bfloat16, lo, hi)
    def permutation(self, n):
        return jax.random.permutation(self._next(), n)


kernel_name = 'parallel_sum__ssm_conv_s4__mixer_channel_mlp__prompt'

def setup_inputs():
    _rng = _Rng(jax.random.key(int.from_bytes(__import__("os").urandom(4), "little")))
    _w = (lambda a: (lambda t: t.astype(jnp.bfloat16) if jnp.issubdtype(t.dtype, jnp.floating) else t)(jnp.asarray(a)))
    def _A_setup():
        B, L, D, N = 1, 2048, 512, 128
        A_re = -jnp.exp((lambda *s: _rng.normal(s) * 0.1)(D, N))
        A_im = jnp.pi * (lambda *s: _rng.normal(s) * 0.1)(D, N)
        B_re = (lambda *s: _rng.normal(s) * 0.1)(D, N)
        B_im = (lambda *s: _rng.normal(s) * 0.1)(D, N)
        C_re = (lambda *s: _rng.normal(s) * 0.1)(D, N)
        C_im = (lambda *s: _rng.normal(s) * 0.1)(D, N)
        log_dt = (lambda *s: _rng.normal(s) * 0.1)(D) * 0.5 - 4.0
        Dskip = (lambda *s: _rng.normal(s) * 0.05)(D)
        return {
            "u": _w((lambda *s: _rng.normal(s) * 0.05)(B, L, D)),
            "A_re": _w(A_re),
            "A_im": _w(A_im),
            "B_re": _w(B_re),
            "B_im": _w(B_im),
            "C_re": _w(C_re),
            "C_im": _w(C_im),
            "log_dt": _w(log_dt),
            "Dskip": _w(Dskip),
        }
    _A_in = _A_setup()

    def _B_setup():
        B, S, D, F = 1, 2048, 512, 1792
        return {
            "x": _w((lambda *s: _rng.normal(s) * 0.05)(B, S, D)),
            "w1": _w((lambda *s: _rng.normal(s) * 0.2)(D, F) * (D ** -0.5)),
            "b1": _w((lambda *s: _rng.normal(s) * 0.2)(F)),
            "w2": _w((lambda *s: _rng.normal(s) * 0.2)(F, D) * (F ** -0.5)),
            "b2": _w((lambda *s: _rng.normal(s) * 0.05)(D)),
        }
    _B_in = _B_setup()

    return {
        "A_u": _A_in["u"],
        "A_A_re": _A_in["A_re"],
        "A_A_im": _A_in["A_im"],
        "A_B_re": _A_in["B_re"],
        "A_B_im": _A_in["B_im"],
        "A_C_re": _A_in["C_re"],
        "A_C_im": _A_in["C_im"],
        "A_log_dt": _A_in["log_dt"],
        "A_Dskip": _A_in["Dskip"],
        "B_x": _B_in["x"],
        "B_w1": _B_in["w1"],
        "B_b1": _B_in["b1"],
        "B_w2": _B_in["w2"],
        "B_b2": _B_in["b2"],
    }

def reference(A_u, A_A_re, A_A_im, A_B_re, A_B_im, A_C_re, A_C_im, A_log_dt, A_Dskip, B_x, B_w1, B_b1, B_w2, B_b2):
    def _A_ref(u, A_re, A_im, B_re, B_im, C_re, C_im, log_dt, Dskip):
        Bsz, L, D = u.shape
        dt = jnp.exp(log_dt)[:, None]
        A = A_re + 1j * A_im
        Bc = B_re + 1j * B_im
        Cc = C_re + 1j * C_im
        logdA = dt * A
        dB = dt * Bc
        l = (lambda x, dt: x.astype(dt))(jnp.arange(L), A_re.dtype)
        P = jnp.exp(logdA[:, :, None] * l[None, None, :])
        K = jnp.einsum("dn,dnl,dn->dl", Cc, P, dB).real
        L2 = 2 * L
        Kp = jnp.pad(K, ((0, 0), (0, L)))
        up = (lambda x, *d: x.transpose(*d))(u, 0, 2, 1)
        up = jnp.pad(up, ((0, 0), (0, 0), (0, L)))
        Kf = (lambda x, axes=(-2,-1): jnp.fft.rfft2(x.astype(jnp.float32), axes=axes))(Kp[:, None, :], axes=(-2, -1))
        Uf = (lambda x, axes=(-2,-1): jnp.fft.rfft2(x.astype(jnp.float32), axes=axes))(up[:, :, None, :], axes=(-2, -1))
        Yf = Uf * Kf[None, :, :, :]
        y = (lambda x, s, axes=(-2,-1): jnp.fft.irfft2(x, s=s, axes=axes).astype(jnp.bfloat16))(Yf, (1, L2), axes=(-2, -1))[:, :, 0, :L]
        y = (lambda x, *d: x.transpose(*d))(y, 0, 2, 1) + u * Dskip[None, None, :]
        return y

    def _B_ref(x, w1, b1, w2, b2):
        y = _layernorm(x, axis=-1)
        h = _gelu(jnp.einsum("bsd,df->bsf", y, w1) + b1)
        return jnp.einsum("bsf,fd->bsd", h, w2) + b2

    x = A_u
    xn = _layernorm(x, axis=-1)
    return x + _A_ref(xn, A_A_re, A_A_im, A_B_re, A_B_im, A_C_re, A_C_im, A_log_dt, A_Dskip) + _B_ref(xn, B_w1, B_b1, B_w2, B_b2)
```

```python
import functools, math
import jax, jax.numpy as jnp, numpy as np
from jax.experimental import pallas as pl
from jax.experimental.pallas import tpu as pltpu

L, D, N, FF = 2048, 512, 128, 1792
NF = 4096
N2 = 16
RP = 136
QR = 24
EPS = 1e-5

RHO = (
    tuple(range(16)),
    (0, 0, 2, 4, 4, 4, 6, 8, 8, 8, 10, 12, 12, 12, 14, 16),
    (0, 0, 0, 4, 4, 4, 8, 8, 8, 8, 8, 12, 12, 12, 16, 16),
    (0, 0, 0, 0, 0, 8, 8, 8, 8, 8, 8, 8, 16, 16, 16, 16),
)
BIN_ROWS = ((0, 16), (16, 32), (32, 64), (64, 128))


def cmul(ar, ai, br, bi):
    return ar * br - ai * bi, ar * bi + ai * br


def _fft16(re, im, sign):
    n = len(re)
    if n == 1:
        return re, im
    er, ei = _fft16(re[0::2], im[0::2], sign)
    orr, oi = _fft16(re[1::2], im[1::2], sign)
    outr = [None] * n
    outi = [None] * n
    for k in range(n // 2):
        ang = sign * 2.0 * math.pi * k / n
        c, s = math.cos(ang), math.sin(ang)
        a_r, a_i = orr[k], oi[k]
        if k == 0:
            tr, ti = a_r, a_i
        elif 4 * k == n:
            if sign < 0:
                tr, ti = a_i, -a_r
            else:
                tr, ti = -a_i, a_r
        else:
            tr = a_r * c - a_i * s
            ti = a_r * s + a_i * c
        outr[k] = er[k] + tr
        outi[k] = ei[k] + ti
        outr[k + n // 2] = er[k] - tr
        outi[k + n // 2] = ei[k] - ti
    return outr, outi


def _layernorm(v):
    m = jnp.mean(v, axis=-1, keepdims=True)
    c = v - m
    var = jnp.mean(c * c, axis=-1, keepdims=True)
    return c * jax.lax.rsqrt(var + EPS)


def _gelu(v):
    return 0.5 * v * (1.0 + jnp.tanh(math.sqrt(2.0 / math.pi) * (v + 0.044715 * (v * v * v))))


def kernel(x_ref, are_ref, aim_ref, bre_ref, bim_ref, cre_ref, cim_ref, ldt_ref, dsk_ref,
           w1_ref, b1_ref, w2_ref, b2_ref, o_ref,
           ai_r, ai_i, bi_r, bi_i, z8_r, z8_i, w8_r, w8_i, g_r, g_i,
           kt, kx, f_scr, g_scr, xs, zx, kh, ys):
    f32, bf16 = jnp.float32, jnp.bfloat16

    row = jax.lax.broadcasted_iota(jnp.int32, (RP, 128), 0)
    lan = jax.lax.broadcasted_iota(jnp.int32, (RP, 128), 1)
    valid = (row <= 128)
    a1 = (-2.0 * math.pi / 256.0) * ((row * lan) & 255).astype(f32)
    t1r = jnp.where(valid, jnp.cos(a1), 0.0); t1i = jnp.where(valid, jnp.sin(a1), 0.0)
    a2 = (-2.0 * math.pi / NF) * (row * lan).astype(f32)
    t2r, t2i = jnp.cos(a2), jnp.sin(a2)
    rowi = jax.lax.broadcasted_iota(jnp.int32, (128, RP), 0)
    lani = jax.lax.broadcasted_iota(jnp.int32, (128, RP), 1)
    wv = jnp.where(lani > 128, 0.0, jnp.where((lani == 0) | (lani == 128), 1.0, 2.0)) * (1.0 / NF)
    b1a = (2.0 * math.pi / 256.0) * ((rowi * lani) & 255).astype(f32)
    s1r = jnp.cos(b1a) * wv; s1i = jnp.sin(b1a) * wv
    b2a = (2.0 * math.pi / NF) * (rowi * lani).astype(f32)
    s2r, s2i = jnp.cos(b2a), jnp.sin(b2a)
    for n2 in range(N2):
        cr_, ci_ = cmul(t1r, t1i, t2r[:, n2:n2 + 1], t2i[:, n2:n2 + 1])
        f_scr[n2, 0:RP, :] = cr_.astype(bf16)
        f_scr[n2, RP:2 * RP, :] = ci_.astype(bf16)
        dr_, di_ = cmul(s1r, s1i, s2r[n2:n2 + 1, :], s2i[n2:n2 + 1, :])
        g_scr[n2, :, 0:RP] = dr_.astype(bf16)
        g_scr[n2, :, RP:2 * RP] = (-di_).astype(bf16)

    dt = jnp.exp(ldt_ref[...].astype(f32)).astype(bf16).astype(f32)
    lr = dt * are_ref[...].astype(f32); li = dt * aim_ref[...].astype(f32)
    dbr = dt * bre_ref[...].astype(f32); dbi = dt * bim_ref[...].astype(f32)
    cr, ci = cmul(cre_ref[...].astype(f32), cim_ref[...].astype(f32), dbr, dbi)
    mg = jnp.exp(lr)
    zr, zi = mg * jnp.cos(li), mg * jnp.sin(li)
    z2r, z2i = cmul(zr, zi, zr, zi); z4r, z4i = cmul(z2r, z2i, z2r, z2i); z8r, z8i = cmul(z4r, z4i, z4r, z4i)
    wr, wi = cmul(z8r, z8i, z8r, z8i)
    ar, ai = cr, ci
    br, bi = jnp.ones_like(wr), jnp.zeros_like(wr)
    for s in range(8):
        ai_r[pl.ds(s, D, stride=8), :] = ar; ai_i[pl.ds(s, D, stride=8), :] = ai
        bi_r[pl.ds(s, D, stride=8), :] = br; bi_i[pl.ds(s, D, stride=8), :] = bi
        ar, ai = cmul(ar, ai, zr, zi)
        br, bi = cmul(br, bi, wr, wi)
    z8_r[...] = z8r; z8_i[...] = z8i
    w8_r[...] = br; w8_i[...] = bi
    gr, gi = br, bi
    for _ in range(3):
        gr, gi = cmul(gr, gi, gr, gi)
    g_r[...] = gr; g_i[...] = gi

    lane24 = jax.lax.broadcasted_iota(jnp.int32, (QR, 128), 1)

    def chan_tables(d):
        o = pl.multiple_of(d * 8, 8)
        a0r = ai_r[pl.ds(o, 8), :]; a0i = ai_i[pl.ds(o, 8), :]
        b0r = bi_r[pl.ds(o, 8), :]; b0i = bi_i[pl.ds(o, 8), :]
        z8r_ = z8_r[pl.ds(d, 1), :]; z8i_ = z8_i[pl.ds(d, 1), :]
        w8r_ = w8_r[pl.ds(d, 1), :]; w8i_ = w8_i[pl.ds(d, 1), :]
        gr_ = g_r[pl.ds(d, 1), :]; gi_ = g_i[pl.ds(d, 1), :]
        a1r, a1i = cmul(a0r, a0i, z8r_, z8i_)
        a2r, a2i = cmul(a1r, a1i, z8r_, z8i_)
        Ar0 = jnp.concatenate([a0r, a1r, a2r], axis=0); Ai0 = jnp.concatenate([a0i, a1i, a2i], axis=0)
        Ar1, Ai1 = cmul(Ar0, Ai0, gr_, gi_)
        Ar = jnp.concatenate([Ar0, Ar1], axis=0); Ai = jnp.concatenate([Ai0, Ai1], axis=0)
        brs = [b0r]; bis = [b0i]
        for _k in range(7):
            r_, i_ = cmul(brs[-1], bis[-1], w8r_, w8i_); brs.append(r_); bis.append(i_)
        return Ar, Ai, jnp.concatenate(brs, axis=0), jnp.concatenate(bis, axis=0)

    def kgen_body(p, carry):
        d0 = 2 * p
        Ar0, Ai0, Br0, Bi0 = chan_tables(d0)
        Ar1, Ai1, Br1, Bi1 = chan_tables(d0 + 1)
        lhs = jnp.concatenate([jnp.concatenate([Ar0, -Ai0], axis=1), jnp.concatenate([Ar1, -Ai1], axis=1)], axis=0).astype(bf16)
        wts = jnp.concatenate([jnp.concatenate([Br0, Bi0], axis=1), jnp.concatenate([Br1, Bi1], axis=1)], axis=0).astype(bf16)
        out = jax.lax.dot_general(lhs, wts, (((1,), (1,)), ((), ())), preferred_element_type=f32)
        t0 = jnp.where(lane24 < 64, out[0:QR], pltpu.roll(out[QR:2 * QR], 64, 1))
        t1 = jnp.where(lane24 < 64, pltpu.roll(out[2 * QR:3 * QR], 64, 1), out[3 * QR:4 * QR])
        kt[pl.ds(pl.multiple_of(d0 * QR, 8), QR), :] = t0
        kt[pl.ds(pl.multiple_of(d0 * QR + QR, 8), QR), :] = t1
        return carry
    jax.lax.fori_loop(0, D // 2, kgen_body, 0)

    for q in range(17):
        kx[q] = kt[pl.ds(q, D, stride=QR), :].T

    for n2 in range(N2):
        parts = [kx[RHO[b][n2], r0:r1, :] for b, (r0, r1) in enumerate(BIN_ROWS)]
        kseg = jnp.concatenate(parts, axis=0).astype(bf16)
        kh[n2] = jnp.dot(f_scr[n2], kseg, preferred_element_type=f32)

    def stageb_k(it, carry):
        rg = it // 4; lt = it % 4
        r0 = pl.multiple_of(rg * 8, 8); c0 = pl.multiple_of(lt * 128, 128)
        re = [kh[n2, pl.ds(r0, 8), pl.ds(c0, 128)] for n2 in range(N2)]
        im = [kh[n2, pl.ds(r0 + RP, 8), pl.ds(c0, 128)] for n2 in range(N2)]
        re, im = _fft16(re, im, -1)
        for f2 in range(N2):
            kh[f2, pl.ds(r0, 8), pl.ds(c0, 128)] = re[f2]
            kh[f2, pl.ds(r0 + RP, 8), pl.ds(c0, 128)] = im[f2]
        return carry
    jax.lax.fori_loop(0, (RP // 8) * 4, stageb_k, 0)

    def ln_body(i, carry):
        r0 = pl.multiple_of(i * 128, 128)
        xv = x_ref[pl.ds(r0, 128), :].astype(f32)
        xn = _layernorm(xv).astype(bf16).astype(f32)
        for dtl in range(4):
            xs[dtl, pl.ds(r0, 128), :] = xn[:, dtl * 128:(dtl + 1) * 128]
        return carry
    jax.lax.fori_loop(0, L // 128, ln_body, 0)

    def sa_body(n2, carry):
        seg = jnp.concatenate([xs[dtl, pl.ds(n2, 128, stride=16), :] for dtl in range(4)], axis=1).astype(bf16)
        zx[n2] = jnp.dot(f_scr[n2], seg, preferred_element_type=f32)
        return carry
    jax.lax.fori_loop(0, N2, sa_body, 0)

    def stageb_x(it, carry):
        rg = it // 4; lt = it % 4
        r0 = pl.multiple_of(rg * 8, 8); c0 = pl.multiple_of(lt * 128, 128)
        re = [zx[n2, pl.ds(r0, 8), pl.ds(c0, 128)] for n2 in range(N2)]
        im = [zx[n2, pl.ds(r0 + RP, 8), pl.ds(c0, 128)] for n2 in range(N2)]
        re, im = _fft16(re, im, -1)
        for f2 in range(N2):
            kr_ = kh[f2, pl.ds(r0, 8), pl.ds(c0, 128)]
            ki_ = kh[f2, pl.ds(r0 + RP, 8), pl.ds(c0, 128)]
            re[f2], im[f2] = cmul(re[f2], im[f2], kr_, ki_)
        re, im = _fft16(re, im, +1)
        for n2 in range(N2):
            zx[n2, pl.ds(r0, 8), pl.ds(c0, 128)] = re[n2]
            zx[n2, pl.ds(r0 + RP, 8), pl.ds(c0, 128)] = im[n2]
        return carry
    jax.lax.fori_loop(0, (RP // 8) * 4, stageb_x, 0)

    def isa_body(n2, carry):
        y = jnp.dot(g_scr[n2], zx[n2].astype(bf16), preferred_element_type=f32)
        for dtl in range(4):
            ys[dtl, pl.ds(n2, 128, stride=16), :] = y[:, dtl * 128:(dtl + 1) * 128]
        return carry
    jax.lax.fori_loop(0, N2, isa_body, 0)

    TM = 256
    def mlp_body(i, carry):
        r0 = pl.multiple_of(i * TM, TM)
        xv = x_ref[pl.ds(r0, TM), :].astype(f32)
        xn = jnp.concatenate([xs[dtl, pl.ds(r0, TM), :] for dtl in range(4)], axis=1)
        yc = jnp.concatenate([ys[dtl, pl.ds(r0, TM), :] for dtl in range(4)], axis=1)
        y2 = _layernorm(xn).astype(bf16)
        h = jnp.dot(y2, w1_ref[...], preferred_element_type=f32) + b1_ref[...].astype(f32)
        h = _gelu(h).astype(bf16)
        o = jnp.dot(h, w2_ref[...], preferred_element_type=f32) + b2_ref[...].astype(f32)
        a_out = yc + xn * dsk_ref[...].astype(f32)
        o_ref[pl.ds(r0, TM), :] = (xv + a_out + o).astype(bf16)
        return carry
    jax.lax.fori_loop(0, L // TM, mlp_body, 0)


@jax.jit
def pallas_parallel_sum__ssm_conv_s4__mixer_channel_mlp__prompt_kernel(A_u, A_A_re, A_A_im, A_B_re, A_B_im, A_C_re, A_C_im, A_log_dt, A_Dskip, B_x, B_w1, B_b1, B_w2, B_b2):
    f32 = jnp.float32
    out = pl.pallas_call(
        kernel,
        out_shape=jax.ShapeDtypeStruct((L, D), jnp.bfloat16),
        scratch_shapes=[pltpu.VMEM((8 * D, N), f32)] * 4 + [pltpu.VMEM((D, N), f32)] * 6 + [
            pltpu.VMEM((D * QR, 128), f32),
            pltpu.VMEM((17, 128, D), f32),
            pltpu.VMEM((N2, 2 * RP, 128), jnp.bfloat16),
            pltpu.VMEM((N2, 128, 2 * RP), jnp.bfloat16),
            pltpu.VMEM((4, L, 128), f32),
            pltpu.VMEM((N2, 2 * RP, D), f32),
            pltpu.VMEM((N2, 2 * RP, D), f32),
            pltpu.VMEM((4, L, 128), f32),
        ],
        compiler_params=pltpu.CompilerParams(vmem_limit_bytes=100 * 1024 * 1024),
    )(A_u.reshape(L, D), A_A_re, A_A_im, A_B_re, A_B_im, A_C_re, A_C_im, A_log_dt.reshape(D, 1),
      A_Dskip.reshape(1, D), B_w1, B_b1.reshape(1, FF), B_w2, B_b2.reshape(1, D))
    return out.reshape(1, L, D)
```

```python
import functools, math
import jax, jax.numpy as jnp, numpy as np
from jax.experimental import pallas as pl
from jax.experimental.pallas import tpu as pltpu

L, D, N, FF = 2048, 512, 128, 1792
NF = 4096
N2 = 16
RP = 136
QR = 24
EPS = 1e-5
UP = 16
TM = 256

RHO = (
    tuple(range(16)),
    (0, 0, 2, 4, 4, 4, 6, 8, 8, 8, 10, 12, 12, 12, 14, 16),
    (0, 0, 0, 4, 4, 4, 8, 8, 8, 8, 8, 12, 12, 12, 16, 16),
    (0, 0, 0, 0, 0, 8, 8, 8, 8, 8, 8, 8, 16, 16, 16, 16),
)
BIN_ROWS = ((0, 16), (16, 32), (32, 64), (64, 128))


def cmul(ar, ai, br, bi):
    return ar * br - ai * bi, ar * bi + ai * br


def _fft16(re, im, sign):
    n = len(re)
    if n == 1:
        return re, im
    er, ei = _fft16(re[0::2], im[0::2], sign)
    orr, oi = _fft16(re[1::2], im[1::2], sign)
    outr = [None] * n
    outi = [None] * n
    for k in range(n // 2):
        ang = sign * 2.0 * math.pi * k / n
        c, s = math.cos(ang), math.sin(ang)
        a_r, a_i = orr[k], oi[k]
        if k == 0:
            tr, ti = a_r, a_i
        elif 4 * k == n:
            if sign < 0:
                tr, ti = a_i, -a_r
            else:
                tr, ti = -a_i, a_r
        else:
            tr = a_r * c - a_i * s
            ti = a_r * s + a_i * c
        outr[k] = er[k] + tr
        outi[k] = ei[k] + ti
        outr[k + n // 2] = er[k] - tr
        outi[k + n // 2] = ei[k] - ti
    return outr, outi


def _layernorm(v):
    m = jnp.mean(v, axis=-1, keepdims=True)
    c = v - m
    var = jnp.mean(c * c, axis=-1, keepdims=True)
    return c * jax.lax.rsqrt(var + EPS)


def _gelu(v):
    return 0.5 * v * (1.0 + jnp.tanh(math.sqrt(2.0 / math.pi) * (v + 0.044715 * (v * v * v))))


def kernel(x_hbm, are_ref, aim_ref, bre_ref, bim_ref, cre_ref, cim_ref, ldt_ref, dsk_ref,
           w1_hbm, b1_ref, w2_hbm, b2_ref, o_hbm,
           ai_r, ai_i, bi_r, bi_i, z8_r, z8_i, w8_r, w8_i, g_r, g_i,
           kt, kx, f_scr, g_scr, xs, zx, kh, ys, part,
           xbuf, w1buf, w2buf, obuf, y2buf, sems):
    f32, bf16 = jnp.float32, jnp.bfloat16

    cp_x = pltpu.make_async_copy(x_hbm, xbuf, sems.at[0]); cp_x.start()
    cp_w1 = pltpu.make_async_copy(w1_hbm, w1buf, sems.at[1]); cp_w1.start()
    cp_w2 = pltpu.make_async_copy(w2_hbm, w2buf, sems.at[2]); cp_w2.start()

    dt = jnp.exp(ldt_ref[...].astype(f32)).astype(bf16).astype(f32)
    lr = dt * are_ref[...].astype(f32); li = dt * aim_ref[...].astype(f32)
    dbr = dt * bre_ref[...].astype(f32); dbi = dt * bim_ref[...].astype(f32)
    cr, ci = cmul(cre_ref[...].astype(f32), cim_ref[...].astype(f32), dbr, dbi)
    mg = jnp.exp(lr)
    zr, zi = mg * jnp.cos(li), mg * jnp.sin(li)
    z2r, z2i = cmul(zr, zi, zr, zi); z4r, z4i = cmul(z2r, z2i, z2r, z2i); z8r, z8i = cmul(z4r, z4i, z4r, z4i)
    wr, wi = cmul(z8r, z8i, z8r, z8i)
    ar, ai = cr, ci
    br, bi = jnp.ones_like(wr), jnp.zeros_like(wr)
    for s in range(8):
        ai_r[pl.ds(s, D, stride=8), :] = ar; ai_i[pl.ds(s, D, stride=8), :] = ai
        bi_r[pl.ds(s, D, stride=8), :] = br; bi_i[pl.ds(s, D, stride=8), :] = bi
        ar, ai = cmul(ar, ai, zr, zi)
        br, bi = cmul(br, bi, wr, wi)
    z8_r[...] = z8r; z8_i[...] = z8i
    w8_r[...] = br; w8_i[...] = bi
    gr, gi = br, bi
    for _ in range(3):
        gr, gi = cmul(gr, gi, gr, gi)
    g_r[...] = gr; g_i[...] = gi

    lane24 = jax.lax.broadcasted_iota(jnp.int32, (QR, 128), 1)

    def chan_tables(d):
        o = pl.multiple_of(d * 8, 8)
        a0r = ai_r[pl.ds(o, 8), :]; a0i = ai_i[pl.ds(o, 8), :]
        b0r = bi_r[pl.ds(o, 8), :]; b0i = bi_i[pl.ds(o, 8), :]
        z8r_ = z8_r[pl.ds(d, 1), :]; z8i_ = z8_i[pl.ds(d, 1), :]
        w8r_ = w8_r[pl.ds(d, 1), :]; w8i_ = w8_i[pl.ds(d, 1), :]
        gr_ = g_r[pl.ds(d, 1), :]; gi_ = g_i[pl.ds(d, 1), :]
        a1r, a1i = cmul(a0r, a0i, z8r_, z8i_)
        a2r, a2i = cmul(a1r, a1i, z8r_, z8i_)
        Ar0 = jnp.concatenate([a0r, a1r, a2r], axis=0); Ai0 = jnp.concatenate([a0i, a1i, a2i], axis=0)
        Ar1, Ai1 = cmul(Ar0, Ai0, gr_, gi_)
        Ar = jnp.concatenate([Ar0, Ar1], axis=0); Ai = jnp.concatenate([Ai0, Ai1], axis=0)
        brs = [b0r]; bis = [b0i]
        for _k in range(7):
            r_, i_ = cmul(brs[-1], bis[-1], w8r_, w8i_); brs.append(r_); bis.append(i_)
        return Ar, Ai, jnp.concatenate(brs, axis=0), jnp.concatenate(bis, axis=0)

    def pow_table(nrow, ncol, base_num, sign, period):
        s8 = jax.lax.broadcasted_iota(jnp.int32, (8, ncol), 0)
        c8 = jax.lax.broadcasted_iota(jnp.int32, (8, ncol), 1)
        ang0 = (sign * 2.0 * math.pi * base_num / period) * (s8 * c8).astype(f32)
        angs = (sign * 2.0 * math.pi * base_num * 8 / period) * c8.astype(f32)
        vr, vi = jnp.cos(ang0), jnp.sin(ang0)
        mr, mi = jnp.cos(angs), jnp.sin(angs)
        rs, is_ = [vr], [vi]
        for _a in range(nrow // 8 - 1):
            vr, vi = cmul(vr, vi, mr, mi)
            rs.append(vr); is_.append(vi)
        return jnp.concatenate(rs, axis=0), jnp.concatenate(is_, axis=0)

    row = jax.lax.broadcasted_iota(jnp.int32, (RP, 128), 0)
    valid = (row <= 128)
    t1r, t1i = pow_table(RP, 128, 1, -1.0, 256.0)
    t1r = jnp.where(valid, t1r, 0.0); t1i = jnp.where(valid, t1i, 0.0)
    t2r, t2i = pow_table(RP, 128, 1, -1.0, float(NF))
    lani = jax.lax.broadcasted_iota(jnp.int32, (128, RP), 1)
    wv = jnp.where(lani > 128, 0.0, jnp.where((lani == 0) | (lani == 128), 1.0, 2.0)) * (1.0 / NF)
    s1r, s1i = pow_table(128, RP, 1, 1.0, 256.0)
    s1r = s1r * wv; s1i = s1i * wv
    s2r, s2i = pow_table(16, RP, 1, 1.0, float(NF))
    for n2 in range(N2):
        cr_, ci_ = cmul(t1r, t1i, t2r[:, n2:n2 + 1], t2i[:, n2:n2 + 1])
        f_scr[n2, 0:RP, :] = cr_.astype(bf16)
        f_scr[n2, RP:2 * RP, :] = ci_.astype(bf16)
        dr_, di_ = cmul(s1r, s1i, s2r[n2:n2 + 1, :], s2i[n2:n2 + 1, :])
        g_scr[n2, :, 0:RP] = dr_.astype(bf16)
        g_scr[n2, :, RP:2 * RP] = (-di_).astype(bf16)

    cp_x.wait()

    def kgen_body(pp, carry):
        for u in range(UP):
            d0 = 2 * (pp * UP + u)
            Ar0, Ai0, Br0, Bi0 = chan_tables(d0)
            Ar1, Ai1, Br1, Bi1 = chan_tables(d0 + 1)
            lhs = jnp.concatenate([jnp.concatenate([Ar0, -Ai0], axis=1), jnp.concatenate([Ar1, -Ai1], axis=1)], axis=0).astype(bf16)
            wts = jnp.concatenate([jnp.concatenate([Br0, Bi0], axis=1), jnp.concatenate([Br1, Bi1], axis=1)], axis=0).astype(bf16)
            out = jax.lax.dot_general(lhs, wts, (((1,), (1,)), ((), ())), preferred_element_type=f32)
            t0 = jnp.where(lane24 < 64, out[0:QR], pltpu.roll(out[QR:2 * QR], 64, 1))
            t1 = jnp.where(lane24 < 64, pltpu.roll(out[2 * QR:3 * QR], 64, 1), out[3 * QR:4 * QR])
            kt[pl.ds(pl.multiple_of(d0 * QR, 8), QR), :] = t0
            kt[pl.ds(pl.multiple_of(d0 * QR + QR, 8), QR), :] = t1
        r0 = pl.multiple_of(pp * 128, 128)
        xv = xbuf[pl.ds(r0, 128), :].astype(f32)
        xn = _layernorm(xv).astype(bf16).astype(f32)
        for dtl in range(4):
            xs[dtl, pl.ds(r0, 128), :] = xn[:, dtl * 128:(dtl + 1) * 128]
        y2buf[pl.ds(r0, 128), :] = _layernorm(xn).astype(bf16)
        return carry
    jax.lax.fori_loop(0, D // 2 // UP, kgen_body, 0)

    for q in range(17):
        kx[q] = kt[pl.ds(q, D, stride=QR), :].T

    for n2 in range(N2):
        parts = [kx[RHO[b][n2], r0:r1, :] for b, (r0, r1) in enumerate(BIN_ROWS)]
        kseg = jnp.concatenate(parts, axis=0).astype(bf16)
        kh[n2] = jnp.dot(f_scr[n2], kseg, preferred_element_type=f32)

    def stageb_k_unit(rg, lt):
        r0 = pl.multiple_of(rg * 8, 8); c0 = lt * 128
        re = [kh[n2, pl.ds(r0, 8), c0:c0 + 128] for n2 in range(N2)]
        im = [kh[n2, pl.ds(r0 + RP, 8), c0:c0 + 128] for n2 in range(N2)]
        re, im = _fft16(re, im, -1)
        for f2 in range(N2):
            kh[f2, pl.ds(r0, 8), c0:c0 + 128] = re[f2]
            kh[f2, pl.ds(r0 + RP, 8), c0:c0 + 128] = im[f2]

    def sa_body(n2h, carry):
        for e in range(2):
            n2 = n2h * 2 + e
            seg = jnp.concatenate([xs[dtl, pl.ds(n2, 128, stride=16), :] for dtl in range(4)], axis=1).astype(bf16)
            zx[n2] = jnp.dot(f_scr[n2], seg, preferred_element_type=f32)
            for lt in range(4):
                stageb_k_unit(n2, lt)
        return carry
    jax.lax.fori_loop(0, N2 // 2, sa_body, 0)
    for lt in range(4):
        stageb_k_unit(16, lt)

    def stageb_x_unit(rg, lt):
        r0 = pl.multiple_of(rg * 8, 8); c0 = lt * 128
        re = [zx[n2, pl.ds(r0, 8), c0:c0 + 128] for n2 in range(N2)]
        im = [zx[n2, pl.ds(r0 + RP, 8), c0:c0 + 128] for n2 in range(N2)]
        re, im = _fft16(re, im, -1)
        for f2 in range(N2):
            kr_ = kh[f2, pl.ds(r0, 8), c0:c0 + 128]
            ki_ = kh[f2, pl.ds(r0 + RP, 8), c0:c0 + 128]
            re[f2], im[f2] = cmul(re[f2], im[f2], kr_, ki_)
        re, im = _fft16(re, im, +1)
        for n2 in range(N2):
            zx[n2, pl.ds(r0, 8), c0:c0 + 128] = re[n2]
            zx[n2, pl.ds(r0 + RP, 8), c0:c0 + 128] = im[n2]

    cp_w1.wait(); cp_w2.wait()

    def mlp_body(i, carry):
        r0 = pl.multiple_of(i * TM, TM)
        xv = xbuf[pl.ds(r0, TM), :].astype(f32)
        xn = jnp.concatenate([xs[dtl, pl.ds(r0, TM), :] for dtl in range(4)], axis=1)
        y2 = y2buf[pl.ds(r0, TM), :]
        h = jnp.dot(y2, w1buf[...], preferred_element_type=f32) + b1_ref[...].astype(f32)
        h = _gelu(h).astype(bf16)
        o = jnp.dot(h, w2buf[...], preferred_element_type=f32) + b2_ref[...].astype(f32)
        part[pl.ds(r0, TM), :] = xv + xn * dsk_ref[...].astype(f32) + o
        for j in range(2):
            for lt in range(4):
                stageb_x_unit(i * 2 + j, lt)
        return carry
    jax.lax.fori_loop(0, L // TM, mlp_body, 0)
    for lt in range(4):
        stageb_x_unit(16, lt)

    def isa_body(n2h, carry):
        for e in range(2):
            n2 = n2h * 2 + e
            y = jnp.dot(g_scr[n2], zx[n2].astype(bf16), preferred_element_type=f32)
            for dtl in range(4):
                ys[dtl, pl.ds(n2, 128, stride=16), :] = y[:, dtl * 128:(dtl + 1) * 128]
        return carry
    jax.lax.fori_loop(0, N2 // 2, isa_body, 0)

    NO = 8
    TO = L // NO
    cps = []
    for c in range(NO):
        r0 = c * TO
        yc = jnp.concatenate([ys[dtl, r0:r0 + TO, :] for dtl in range(4)], axis=1)
        obuf[r0:r0 + TO, :] = (part[r0:r0 + TO, :] + yc).astype(bf16)
        cp = pltpu.make_async_copy(obuf.at[r0:r0 + TO, :], o_hbm.at[r0:r0 + TO, :], sems.at[3 + c])
        cp.start(); cps.append(cp)
    for cp in cps:
        cp.wait()


@jax.jit
def pallas_parallel_sum__ssm_conv_s4__mixer_channel_mlp__prompt_kernel(A_u, A_A_re, A_A_im, A_B_re, A_B_im, A_C_re, A_C_im, A_log_dt, A_Dskip, B_x, B_w1, B_b1, B_w2, B_b2):
    f32 = jnp.float32
    anyspec = pl.BlockSpec(memory_space=pl.ANY)
    vm = pl.BlockSpec(memory_space=pltpu.VMEM)
    out = pl.pallas_call(
        kernel,
        out_shape=jax.ShapeDtypeStruct((L, D), jnp.bfloat16),
        in_specs=[anyspec, vm, vm, vm, vm, vm, vm, vm, vm, anyspec, vm, anyspec, vm],
        out_specs=anyspec,
        scratch_shapes=[pltpu.VMEM((8 * D, N), f32)] * 4 + [pltpu.VMEM((D, N), f32)] * 6 + [
            pltpu.VMEM((D * QR, 128), f32),
            pltpu.VMEM((17, 128, D), f32),
            pltpu.VMEM((N2, 2 * RP, 128), jnp.bfloat16),
            pltpu.VMEM((N2, 128, 2 * RP), jnp.bfloat16),
            pltpu.VMEM((4, L, 128), f32),
            pltpu.VMEM((N2, 2 * RP, D), f32),
            pltpu.VMEM((N2, 2 * RP, D), f32),
            pltpu.VMEM((4, L, 128), f32),
            pltpu.VMEM((L, D), f32),
            pltpu.VMEM((L, D), jnp.bfloat16),
            pltpu.VMEM((D, FF), jnp.bfloat16),
            pltpu.VMEM((FF, D), jnp.bfloat16),
            pltpu.VMEM((L, D), jnp.bfloat16),
            pltpu.VMEM((L, D), jnp.bfloat16),
            pltpu.SemaphoreType.DMA((11,)),
        ],
        compiler_params=pltpu.CompilerParams(vmem_limit_bytes=110 * 1024 * 1024),
    )(A_u.reshape(L, D), A_A_re, A_A_im, A_B_re, A_B_im, A_C_re, A_C_im, A_log_dt.reshape(D, 1),
      A_Dskip.reshape(1, D), B_w1, B_b1.reshape(1, FF), B_w2, B_b2.reshape(1, D))
    return out.reshape(1, L, D)
```

```python
import functools, math
import jax, jax.numpy as jnp, numpy as np
from jax.experimental import pallas as pl
from jax.experimental.pallas import tpu as pltpu

L, D, N, FF = 2048, 512, 128, 1792
NF = 4096
N2 = 16
RP = 136
QR = 24
EPS = 1e-5
UP = 16
TM = 256

RHO = (
    tuple(range(16)),
    (0, 0, 2, 4, 4, 4, 6, 8, 8, 8, 10, 12, 12, 12, 14, 16),
    (0, 0, 0, 4, 4, 4, 8, 8, 8, 8, 8, 12, 12, 12, 16, 16),
    (0, 0, 0, 0, 0, 8, 8, 8, 8, 8, 8, 8, 16, 16, 16, 16),
)
BIN_ROWS = ((0, 16), (16, 32), (32, 64), (64, 128))


def cmul(ar, ai, br, bi):
    return ar * br - ai * bi, ar * bi + ai * br


def _fft16(re, im, sign):
    n = len(re)
    if n == 1:
        return re, im
    er, ei = _fft16(re[0::2], im[0::2], sign)
    orr, oi = _fft16(re[1::2], im[1::2], sign)
    outr = [None] * n
    outi = [None] * n
    for k in range(n // 2):
        ang = sign * 2.0 * math.pi * k / n
        c, s = math.cos(ang), math.sin(ang)
        a_r, a_i = orr[k], oi[k]
        if k == 0:
            tr, ti = a_r, a_i
        elif 4 * k == n:
            if sign < 0:
                tr, ti = a_i, -a_r
            else:
                tr, ti = -a_i, a_r
        else:
            tr = a_r * c - a_i * s
            ti = a_r * s + a_i * c
        outr[k] = er[k] + tr
        outi[k] = ei[k] + ti
        outr[k + n // 2] = er[k] - tr
        outi[k + n // 2] = ei[k] - ti
    return outr, outi


def _layernorm(v):
    m = jnp.mean(v, axis=-1, keepdims=True)
    c = v - m
    var = jnp.mean(c * c, axis=-1, keepdims=True)
    return c * jax.lax.rsqrt(var + EPS)


def _gelu(v):
    return 0.5 * v * (1.0 + jnp.tanh(math.sqrt(2.0 / math.pi) * (v + 0.044715 * (v * v * v))))


def kernel(x_hbm, are_ref, aim_ref, bre_ref, bim_ref, cre_ref, cim_ref, ldt_ref, dsk_ref,
           w1_hbm, b1_ref, w2_hbm, b2_ref, o_hbm,
           ai_r, ai_i, bi_r, bi_i, z8_r, z8_i, w8_r, w8_i, g_r, g_i,
           kt, kx, f_scr, g_scr, xs, zx, kh, ys, part,
           xbuf, w1buf, w2buf, obuf, y2buf, sems):
    f32, bf16 = jnp.float32, jnp.bfloat16

    cp_x = pltpu.make_async_copy(x_hbm, xbuf, sems.at[0]); cp_x.start()
    cp_w1 = pltpu.make_async_copy(w1_hbm, w1buf, sems.at[1]); cp_w1.start()
    cp_w2 = pltpu.make_async_copy(w2_hbm, w2buf, sems.at[2]); cp_w2.start()

    dt = jnp.exp(ldt_ref[...].astype(f32).reshape(D, 1)).astype(bf16).astype(f32)
    lr = dt * are_ref[...].astype(f32); li = dt * aim_ref[...].astype(f32)
    dbr = dt * bre_ref[...].astype(f32); dbi = dt * bim_ref[...].astype(f32)
    cr, ci = cmul(cre_ref[...].astype(f32), cim_ref[...].astype(f32), dbr, dbi)
    mg = jnp.exp(lr)
    zr, zi = mg * jnp.cos(li), mg * jnp.sin(li)
    z2r, z2i = cmul(zr, zi, zr, zi); z4r, z4i = cmul(z2r, z2i, z2r, z2i); z8r, z8i = cmul(z4r, z4i, z4r, z4i)
    wr, wi = cmul(z8r, z8i, z8r, z8i)
    ar, ai = cr, ci
    br, bi = jnp.ones_like(wr), jnp.zeros_like(wr)
    for s in range(8):
        ai_r[pl.ds(s, D, stride=8), :] = ar; ai_i[pl.ds(s, D, stride=8), :] = ai
        bi_r[pl.ds(s, D, stride=8), :] = br; bi_i[pl.ds(s, D, stride=8), :] = bi
        ar, ai = cmul(ar, ai, zr, zi)
        br, bi = cmul(br, bi, wr, wi)
    z8_r[...] = z8r; z8_i[...] = z8i
    w8_r[...] = br; w8_i[...] = bi
    gr, gi = br, bi
    for _ in range(3):
        gr, gi = cmul(gr, gi, gr, gi)
    g_r[...] = gr; g_i[...] = gi

    lane24 = jax.lax.broadcasted_iota(jnp.int32, (QR, 128), 1)

    def chan_tables(d):
        o = pl.multiple_of(d * 8, 8)
        a0r = ai_r[pl.ds(o, 8), :]; a0i = ai_i[pl.ds(o, 8), :]
        b0r = bi_r[pl.ds(o, 8), :]; b0i = bi_i[pl.ds(o, 8), :]
        z8r_ = z8_r[pl.ds(d, 1), :]; z8i_ = z8_i[pl.ds(d, 1), :]
        w8r_ = w8_r[pl.ds(d, 1), :]; w8i_ = w8_i[pl.ds(d, 1), :]
        gr_ = g_r[pl.ds(d, 1), :]; gi_ = g_i[pl.ds(d, 1), :]
        a1r, a1i = cmul(a0r, a0i, z8r_, z8i_)
        a2r, a2i = cmul(a1r, a1i, z8r_, z8i_)
        Ar0 = jnp.concatenate([a0r, a1r, a2r], axis=0); Ai0 = jnp.concatenate([a0i, a1i, a2i], axis=0)
        Ar1, Ai1 = cmul(Ar0, Ai0, gr_, gi_)
        Ar = jnp.concatenate([Ar0, Ar1], axis=0); Ai = jnp.concatenate([Ai0, Ai1], axis=0)
        brs = [b0r]; bis = [b0i]
        for _k in range(7):
            r_, i_ = cmul(brs[-1], bis[-1], w8r_, w8i_); brs.append(r_); bis.append(i_)
        return Ar, Ai, jnp.concatenate(brs, axis=0), jnp.concatenate(bis, axis=0)

    def pow_table(nrow, ncol, base_num, sign, period):
        s8 = jax.lax.broadcasted_iota(jnp.int32, (8, ncol), 0)
        c8 = jax.lax.broadcasted_iota(jnp.int32, (8, ncol), 1)
        ang0 = (sign * 2.0 * math.pi * base_num / period) * (s8 * c8).astype(f32)
        angs = (sign * 2.0 * math.pi * base_num * 8 / period) * c8.astype(f32)
        vr, vi = jnp.cos(ang0), jnp.sin(ang0)
        mr, mi = jnp.cos(angs), jnp.sin(angs)
        rs, is_ = [vr], [vi]
        for _a in range(nrow // 8 - 1):
            vr, vi = cmul(vr, vi, mr, mi)
            rs.append(vr); is_.append(vi)
        return jnp.concatenate(rs, axis=0), jnp.concatenate(is_, axis=0)

    row = jax.lax.broadcasted_iota(jnp.int32, (RP, 128), 0)
    valid = (row <= 128)
    t1r, t1i = pow_table(RP, 128, 1, -1.0, 256.0)
    t1r = jnp.where(valid, t1r, 0.0); t1i = jnp.where(valid, t1i, 0.0)
    t2r, t2i = pow_table(RP, 128, 1, -1.0, float(NF))
    lani = jax.lax.broadcasted_iota(jnp.int32, (128, RP), 1)
    wv = jnp.where(lani > 128, 0.0, jnp.where((lani == 0) | (lani == 128), 1.0, 2.0)) * (1.0 / NF)
    s1r, s1i = pow_table(128, RP, 1, 1.0, 256.0)
    s1r = s1r * wv; s1i = s1i * wv
    s2r, s2i = pow_table(16, RP, 1, 1.0, float(NF))
    for n2 in range(N2):
        cr_, ci_ = cmul(t1r, t1i, t2r[:, n2:n2 + 1], t2i[:, n2:n2 + 1])
        f_scr[n2, 0:RP, :] = cr_.astype(bf16)
        f_scr[n2, RP:2 * RP, :] = ci_.astype(bf16)
        dr_, di_ = cmul(s1r, s1i, s2r[n2:n2 + 1, :], s2i[n2:n2 + 1, :])
        g_scr[n2, :, 0:RP] = dr_.astype(bf16)
        g_scr[n2, :, RP:2 * RP] = (-di_).astype(bf16)

    cp_x.wait()

    def kgen_body(pp, carry):
        for u in range(UP):
            d0 = 2 * (pp * UP + u)
            Ar0, Ai0, Br0, Bi0 = chan_tables(d0)
            Ar1, Ai1, Br1, Bi1 = chan_tables(d0 + 1)
            lhs = jnp.concatenate([jnp.concatenate([Ar0, -Ai0], axis=1), jnp.concatenate([Ar1, -Ai1], axis=1)], axis=0).astype(bf16)
            wts = jnp.concatenate([jnp.concatenate([Br0, Bi0], axis=1), jnp.concatenate([Br1, Bi1], axis=1)], axis=0).astype(bf16)
            out = jax.lax.dot_general(lhs, wts, (((1,), (1,)), ((), ())), preferred_element_type=f32)
            t0 = jnp.where(lane24 < 64, out[0:QR], pltpu.roll(out[QR:2 * QR], 64, 1))
            t1 = jnp.where(lane24 < 64, pltpu.roll(out[2 * QR:3 * QR], 64, 1), out[3 * QR:4 * QR])
            kt[pl.ds(pl.multiple_of(d0 * QR, 8), QR), :] = t0
            kt[pl.ds(pl.multiple_of(d0 * QR + QR, 8), QR), :] = t1
        r0 = pl.multiple_of(pp * 128, 128)
        xv = xbuf[pl.ds(r0, 128), :].astype(f32)
        xn = _layernorm(xv).astype(bf16).astype(f32)
        for dtl in range(4):
            xs[dtl, pl.ds(r0, 128), :] = xn[:, dtl * 128:(dtl + 1) * 128]
        y2buf[pl.ds(r0, 128), :] = _layernorm(xn).astype(bf16)
        return carry
    jax.lax.fori_loop(0, D // 2 // UP, kgen_body, 0)

    for q in range(17):
        kx[q] = kt[pl.ds(q, D, stride=QR), :].T

    for n2 in range(N2):
        parts = [kx[RHO[b][n2], r0:r1, :] for b, (r0, r1) in enumerate(BIN_ROWS)]
        kseg = jnp.concatenate(parts, axis=0).astype(bf16)
        kh[n2] = jnp.dot(f_scr[n2], kseg, preferred_element_type=f32)

    def stageb_k_unit(rg, lt):
        r0 = pl.multiple_of(rg * 8, 8); c0 = lt * 128
        re = [kh[n2, pl.ds(r0, 8), c0:c0 + 128] for n2 in range(N2)]
        im = [kh[n2, pl.ds(r0 + RP, 8), c0:c0 + 128] for n2 in range(N2)]
        re, im = _fft16(re, im, -1)
        for f2 in range(N2):
            kh[f2, pl.ds(r0, 8), c0:c0 + 128] = re[f2]
            kh[f2, pl.ds(r0 + RP, 8), c0:c0 + 128] = im[f2]

    def sa_body(n2h, carry):
        for e in range(2):
            n2 = n2h * 2 + e
            seg = jnp.concatenate([xs[dtl, pl.ds(n2, 128, stride=16), :] for dtl in range(4)], axis=1).astype(bf16)
            zx[n2] = jnp.dot(f_scr[n2], seg, preferred_element_type=f32)
            for lt in range(4):
                stageb_k_unit(n2, lt)
        return carry
    jax.lax.fori_loop(0, N2 // 2, sa_body, 0)
    for lt in range(4):
        stageb_k_unit(16, lt)

    def stageb_x_unit(rg, lt):
        r0 = pl.multiple_of(rg * 8, 8); c0 = lt * 128
        re = [zx[n2, pl.ds(r0, 8), c0:c0 + 128] for n2 in range(N2)]
        im = [zx[n2, pl.ds(r0 + RP, 8), c0:c0 + 128] for n2 in range(N2)]
        re, im = _fft16(re, im, -1)
        for f2 in range(N2):
            kr_ = kh[f2, pl.ds(r0, 8), c0:c0 + 128]
            ki_ = kh[f2, pl.ds(r0 + RP, 8), c0:c0 + 128]
            re[f2], im[f2] = cmul(re[f2], im[f2], kr_, ki_)
        re, im = _fft16(re, im, +1)
        for n2 in range(N2):
            zx[n2, pl.ds(r0, 8), c0:c0 + 128] = re[n2]
            zx[n2, pl.ds(r0 + RP, 8), c0:c0 + 128] = im[n2]

    cp_w1.wait(); cp_w2.wait()

    def mlp_body(i, carry):
        r0 = pl.multiple_of(i * TM, TM)
        xv = xbuf[pl.ds(r0, TM), :].astype(f32)
        xn = jnp.concatenate([xs[dtl, pl.ds(r0, TM), :] for dtl in range(4)], axis=1)
        y2 = y2buf[pl.ds(r0, TM), :]
        h = jnp.dot(y2, w1buf[...], preferred_element_type=f32) + b1_ref[...].astype(f32).reshape(1, FF)
        h = _gelu(h).astype(bf16)
        o = jnp.dot(h, w2buf[...], preferred_element_type=f32) + b2_ref[...].astype(f32).reshape(1, D)
        part[pl.ds(r0, TM), :] = xv + xn * dsk_ref[...].astype(f32).reshape(1, D) + o
        for j in range(2):
            for lt in range(4):
                stageb_x_unit(i * 2 + j, lt)
        return carry
    jax.lax.fori_loop(0, L // TM, mlp_body, 0)
    for lt in range(4):
        stageb_x_unit(16, lt)

    def isa_body(n2h, carry):
        for e in range(2):
            n2 = n2h * 2 + e
            y = jnp.dot(g_scr[n2], zx[n2].astype(bf16), preferred_element_type=f32)
            for dtl in range(4):
                ys[dtl, pl.ds(n2, 128, stride=16), :] = y[:, dtl * 128:(dtl + 1) * 128]
        return carry
    jax.lax.fori_loop(0, N2 // 2, isa_body, 0)

    NO = 8
    TO = L // NO
    cps = []
    for c in range(NO):
        r0 = c * TO
        yc = jnp.concatenate([ys[dtl, r0:r0 + TO, :] for dtl in range(4)], axis=1)
        obuf[r0:r0 + TO, :] = (part[r0:r0 + TO, :] + yc).astype(bf16)
        cp = pltpu.make_async_copy(obuf.at[r0:r0 + TO, :], o_hbm.at[r0:r0 + TO, :], sems.at[3 + c])
        cp.start(); cps.append(cp)
    for cp in cps:
        cp.wait()


@jax.jit
def pallas_parallel_sum__ssm_conv_s4__mixer_channel_mlp__prompt_kernel(A_u, A_A_re, A_A_im, A_B_re, A_B_im, A_C_re, A_C_im, A_log_dt, A_Dskip, B_x, B_w1, B_b1, B_w2, B_b2):
    f32 = jnp.float32
    anyspec = pl.BlockSpec(memory_space=pl.ANY)
    vm = pl.BlockSpec(memory_space=pltpu.VMEM)
    out = pl.pallas_call(
        kernel,
        out_shape=jax.ShapeDtypeStruct((L, D), jnp.bfloat16),
        in_specs=[anyspec, vm, vm, vm, vm, vm, vm, vm, vm, anyspec, vm, anyspec, vm],
        out_specs=anyspec,
        scratch_shapes=[pltpu.VMEM((8 * D, N), f32)] * 4 + [pltpu.VMEM((D, N), f32)] * 6 + [
            pltpu.VMEM((D * QR, 128), f32),
            pltpu.VMEM((17, 128, D), f32),
            pltpu.VMEM((N2, 2 * RP, 128), jnp.bfloat16),
            pltpu.VMEM((N2, 128, 2 * RP), jnp.bfloat16),
            pltpu.VMEM((4, L, 128), f32),
            pltpu.VMEM((N2, 2 * RP, D), f32),
            pltpu.VMEM((N2, 2 * RP, D), f32),
            pltpu.VMEM((4, L, 128), f32),
            pltpu.VMEM((L, D), f32),
            pltpu.VMEM((L, D), jnp.bfloat16),
            pltpu.VMEM((D, FF), jnp.bfloat16),
            pltpu.VMEM((FF, D), jnp.bfloat16),
            pltpu.VMEM((L, D), jnp.bfloat16),
            pltpu.VMEM((L, D), jnp.bfloat16),
            pltpu.SemaphoreType.DMA((11,)),
        ],
        compiler_params=pltpu.CompilerParams(vmem_limit_bytes=110 * 1024 * 1024),
    )(A_u.reshape(L, D), A_A_re, A_A_im, A_B_re, A_B_im, A_C_re, A_C_im, A_log_dt,
      A_Dskip, B_w1, B_b1, B_w2, B_b2)
    return out.reshape(1, L, D)
```
